```python
import jax
import jax.numpy as jnp

def _softmax(x, axis=-1):
    return jax.nn.softmax(x, axis=axis)
def _gelu(x):
    return jax.nn.gelu(x, approximate=True)
def _silu(x):
    return jax.nn.silu(x)
def _sigmoid(x):
    return jax.nn.sigmoid(x)
def _layernorm(x, axis=-1, eps=1e-5):
    m = jnp.mean(x, axis=axis, keepdims=True)
    v = jnp.var(x, axis=axis, keepdims=True)
    return (x - m) / jnp.sqrt(v + eps)
def _scatter_add(tgt, idx, src, axis=0):
    return tgt.at[idx].add(src)
def _segment_sum(src, seg, n):
    return jax.ops.segment_sum(src, seg, n)
class _Rng:
    def __init__(self, key):
        self._k = key
    def _next(self):
        self._k, sub = jax.random.split(self._k)
        return sub
    def normal(self, shape):
        return jax.random.normal(self._next(), shape, dtype=jnp.bfloat16)
    def randint(self, lo, hi, shape):
        return jax.random.randint(self._next(), shape, lo, hi, dtype=jnp.int32)
    def uniform(self, shape, lo=0.0, hi=1.0):
        return jax.random.uniform(self._next(), shape, jnp.bfloat16, lo, hi)
    def permutation(self, n):
        return jax.random.permutation(self._next(), n)


kernel_name = 'concat_heads__ssm_conv_h3__compressed_kv_cla__prompt'

def setup_inputs():
    _rng = _Rng(jax.random.key(int.from_bytes(__import__("os").urandom(4), "little")))
    _w = (lambda a: (lambda t: t.astype(jnp.bfloat16) if jnp.issubdtype(t.dtype, jnp.floating) else t)(jnp.asarray(a)))
    def _A_setup():
        B, S, D = 1, 2048, 448
        ks = 4
        return {
            "q": _w((lambda *s: _rng.normal(s) * 0.05)(B, S, D)),
            "k": _w((lambda *s: _rng.normal(s) * 0.05)(B, S, D)),
            "v": _w((lambda *s: _rng.normal(s) * 0.05)(B, S, D)),
            "shift_k": _w((lambda *s: _rng.normal(s) * 0.05)(D, ks) * 0.5),
            "ssm_k": _w((lambda *s: _rng.normal(s) * 0.05)(D, S) * (1.0 / S ** 0.5)),
            "ssm_D": _w((lambda *s: _rng.normal(s) * 0.05)(D)),
        }
    _A_in = _A_setup()

    def _B_setup():
        B, H, Sq, Sk, D, M = 1, 16, 2048, 2048, 256, 448
        Dc = 4 * D
        return {
            "x": _w((lambda *s: _rng.normal(s) * 0.05)(B, Sq, M)),
            "c_kv": _w((lambda *s: _rng.normal(s) * 0.05)(B, Sk, Dc)),
            "w_q": _w((lambda *s: _rng.normal(s) * 0.05)(M, H, D) * (M ** -0.5)),
            "w_uk": _w((lambda *s: _rng.normal(s) * 0.05)(Dc, H, D) * (Dc ** -0.5)),
            "w_uv": _w((lambda *s: _rng.normal(s) * 0.05)(Dc, H, D) * (Dc ** -0.5)),
            "w_o": _w((lambda *s: _rng.normal(s) * 0.05)(H, D, M) * ((H * D) ** -0.5)),
        }
    _B_in = _B_setup()

    return {
        "A_q": _A_in["q"],
        "A_k": _A_in["k"],
        "A_v": _A_in["v"],
        "A_shift_k": _A_in["shift_k"],
        "A_ssm_k": _A_in["ssm_k"],
        "A_ssm_D": _A_in["ssm_D"],
        "B_x": _B_in["x"],
        "B_c_kv": _B_in["c_kv"],
        "B_w_q": _B_in["w_q"],
        "B_w_uk": _B_in["w_uk"],
        "B_w_uv": _B_in["w_uv"],
        "B_w_o": _B_in["w_o"],
    }

def reference(A_q, A_k, A_v, A_shift_k, A_ssm_k, A_ssm_D, B_x, B_c_kv, B_w_q, B_w_uk, B_w_uv, B_w_o):
    def _A_ref(q, k, v, shift_k, ssm_k, ssm_D):
        B, S, D = q.shape
        ks = shift_k.shape[-1]
        k_pad = jnp.pad(k, ((0, 0), (ks - 1, 0), (0, 0)))
        k_shift = jnp.zeros_like(k)
        for t in range(ks):
            k_shift = k_shift + k_pad[:, t:t + S, :] * shift_k[:, ks - 1 - t][None, None, :]
        kv = k_shift * v
        L = 2 * S
        kv_pad = jnp.pad(kv, ((0, 0), (0, S), (0, 0)))
        kf_pad = jnp.pad(ssm_k, ((0, 0), (0, S)))
        kv_f = (lambda x, axes=(-2,-1): jnp.fft.rfft2(x.astype(jnp.float32), axes=axes))(kv_pad[:, None, :, :], axes=(1, 2))
        kf_f = (lambda x, axes=(-2,-1): jnp.fft.rfft2(x.astype(jnp.float32), axes=axes))(kf_pad[:, None, :], axes=(1, 2))
        kf_f = (lambda x, *d: x.transpose(*d))(kf_f, 1, 2, 0)
        y_f = kv_f * kf_f[None, :, :, :]
        y = (lambda x, s, axes=(-2,-1): jnp.fft.irfft2(x, s=s, axes=axes).astype(jnp.bfloat16))(y_f, (1, L), axes=(1, 2))[:, 0, :S, :]
        y = y + kv * ssm_D[None, None, :]
        return q * y

    def _B_ref(x, c_kv, w_q, w_uk, w_uv, w_o):
        B, Sq, M = x.shape[0], x.shape[1], x.shape[2]
        Sk = c_kv.shape[1]
        H, D = w_q.shape[1], w_q.shape[2]
        q = jnp.einsum("bqm,mhd->bhqd", x, w_q)
        k = jnp.einsum("bkc,chd->bhkd", c_kv, w_uk)
        v = jnp.einsum("bkc,chd->bhkd", c_kv, w_uv)
        scores = jnp.einsum("bhqd,bhkd->bhqk", q, k) * (D ** -0.5)
        off = Sk - Sq
        qi = jnp.arange(Sq)[:, None]
        kj = jnp.arange(Sk)[None, :]
        cmask = kj <= (qi + off)
        scores = jnp.where(cmask[None, None], scores, -1e9)
        p = _softmax(scores, axis=-1)
        ctx = jnp.einsum("bhqk,bhkd->bhqd", p, v)
        return jnp.einsum("bhqd,hdm->bqm", ctx, w_o)

    a = _A_ref(A_q, A_k, A_v, A_shift_k, A_ssm_k, A_ssm_D)
    b = _B_ref(B_x, B_c_kv, B_w_q, B_w_uk, B_w_uv, B_w_o)
    return jnp.concatenate([a, b], axis=-1)
```

```python
import numpy as np
import jax
import jax.numpy as jnp
from jax import lax
import jax.experimental.pallas as pl
import jax.experimental.pallas.tpu as pltpu

S, DA, H, D, M, DC = 2048, 448, 16, 256, 448, 1024
C = 128
NC = S // C
BQ = 256
f32, bf16 = jnp.float32, jnp.bfloat16
NT = (((1,), (1,)), ((), ()))


def _dft():
    n = np.arange(C)[None, :]
    f = np.arange(C)[:, None]
    ang = 2 * np.pi * f * n / (2 * C)
    fw = np.concatenate([np.cos(ang), -np.sin(ang)], 0)
    fw[C] = np.cos(np.pi * n[0])
    t = np.arange(2 * C)[:, None]
    fr = np.arange(C)[None, :]
    a2 = 2 * np.pi * t * fr / (2 * C)
    ic = 2 * np.cos(a2)
    ic[:, 0] = 1
    isn = -2 * np.sin(a2)
    isn[:, 0] = np.cos(np.pi * t[:, 0])
    inv = np.concatenate([ic, isn], 1) / (2 * C)
    inv2 = np.concatenate([inv[:C], inv[C:]], 1)
    return fw.astype(np.float32), inv2.astype(np.float32)


def _head(wref, hp):
    w = wref.bitcast(jnp.uint32)[:, hp, :]
    lo = lax.bitcast_convert_type(w << 16, f32).astype(bf16)
    hi = lax.bitcast_convert_type(w & jnp.uint32(0xFFFF0000), f32).astype(bf16)
    return lo, hi


def _kernel(aq, ak, av, sh, sk, sd, fw, inv, x, c, wq, wuk, wuv, wo, out,
            kpad, kvs, U, K, Z, q_s, k_s, v_s, s_s, ctx_s, acc):
    p = pl.program_id(0)

    @pl.when(p == 0)
    def _():
        kpad[0:8, :] = jnp.zeros((8, DA), f32)
        kpad[8:, :] = ak[...].astype(f32)
        acc[...] = jnp.zeros_like(acc)
        Z[0] = jnp.zeros((2 * C, DA), bf16)
        F = fw[...]
        for ch in range(NC):
            ks = jnp.zeros((C, DA), bf16)
            for t in range(4):
                j = 3 - t
                ks = ks + kpad[8 + ch * C - j: 8 + (ch + 1) * C - j, :].astype(bf16) * sh[j:j + 1, :]
            kv = ks * av[ch * C:(ch + 1) * C, :]
            kvs[ch * C:(ch + 1) * C, :] = kv
            U[ch] = jnp.dot(F, kv, preferred_element_type=f32)
            K[ch] = lax.dot_general(F, sk[:, ch * C:(ch + 1) * C], NT, preferred_element_type=f32)

    row0 = lax.broadcasted_iota(jnp.int32, (C, DA), 0) == 0
    for e in range(2):
        ch = 2 * p + e

        def body(d, carry):
            zr, zi = carry
            kr, ki = K[d, :C, :], K[d, C:, :]
            ur, ui = U[ch - d, :C, :], U[ch - d, C:, :]
            ii = ki * ui
            zr = zr + kr * ur - jnp.where(row0, 0.0, ii)
            zi = zi + jnp.where(row0, ii, kr * ui + ki * ur)
            return zr, zi
        z0 = jnp.zeros((C, DA), f32)
        zr, zi = lax.fori_loop(0, ch + 1, body, (z0, z0))
        Z[ch + 1, :C, :] = zr.astype(bf16)
        Z[ch + 1, C:, :] = zi.astype(bf16)
        y = (jnp.dot(inv[:, :2 * C], Z[ch + 1], preferred_element_type=f32)
             + jnp.dot(inv[:, 2 * C:], Z[ch], preferred_element_type=f32)).astype(bf16)
        r = pl.ds(pl.multiple_of(ch * C, C), C)
        y = y + kvs[r, :] * sd[...]
        out[r, :DA] = aq[r, :] * y

    wqs, wks, wvs = _head(wq, p), _head(wuk, p), _head(wuv, p)
    tri = (lax.broadcasted_iota(jnp.int32, (BQ, BQ), 1) <= lax.broadcasted_iota(jnp.int32, (BQ, BQ), 0))
    for e in range(2):
        q_s[...] = (jnp.dot(x[...], wqs[e], preferred_element_type=f32).astype(bf16) * (D ** -0.5)).astype(bf16)
        k_s[...] = jnp.dot(c[...], wks[e], preferred_element_type=f32).astype(bf16)
        v_s[...] = jnp.dot(c[...], wvs[e], preferred_element_type=f32).astype(bf16)
        for i in range(S // BQ):
            n = (i + 1) * BQ
            qi = q_s[i * BQ:(i + 1) * BQ, :]
            s = lax.dot_general(qi, k_s[:n, :], NT, preferred_element_type=f32)
            sd_ = jnp.where(tri, s[:, n - BQ:], -1e9)
            s = sd_ if i == 0 else jnp.concatenate([s[:, :n - BQ], sd_], 1)
            m = jnp.max(s, -1, keepdims=True)
            pe = jnp.exp(s - m)
            l = jnp.sum(pe, -1, keepdims=True)
            o = jnp.dot(pe.astype(bf16), v_s[:n, :], preferred_element_type=f32)
            ctx_s[i * BQ:(i + 1) * BQ, :] = (o * (1.0 / l)).astype(bf16)
        acc[...] += jnp.dot(ctx_s[...], wo[e], preferred_element_type=f32)

    @pl.when(p == H // 2 - 1)
    def _():
        out[:, DA:] = acc[...].astype(bf16)


@jax.jit
def pallas_concat_heads__ssm_conv_h3__compressed_kv_cla__prompt_kernel(
        A_q, A_k, A_v, A_shift_k, A_ssm_k, A_ssm_D, B_x, B_c_kv, B_w_q, B_w_uk, B_w_uv, B_w_o):
    fw, inv = _dft()
    fw, inv = jnp.asarray(fw, bf16), jnp.asarray(inv, bf16)

    def full(a):
        nd = a.ndim
        return pl.BlockSpec(a.shape, lambda p: (0,) * nd, pipeline_mode=pl.Buffered(1))
    args = [A_q[0], A_k[0], A_v[0], A_shift_k.T, A_ssm_k, A_ssm_D[None, :], fw, inv,
            B_x[0], B_c_kv[0], B_w_q, B_w_uk, B_w_uv]
    V = pltpu.VMEM
    o = pl.pallas_call(
        _kernel,
        grid=(H // 2,),
        in_specs=[full(a) for a in args] + [pl.BlockSpec((2, D, M), lambda p: (p, 0, 0))],
        out_specs=pl.BlockSpec((S, DA + M), lambda p: (0, 0)),
        out_shape=jax.ShapeDtypeStruct((S, DA + M), bf16),
        scratch_shapes=[V((S + 8, DA), f32), V((S, DA), bf16), V((NC, 2 * C, DA), f32),
                        V((NC, 2 * C, DA), f32), V((NC + 1, 2 * C, DA), bf16),
                        V((S, D), bf16), V((S, D), bf16), V((S, D), bf16), V((BQ, S), f32),
                        V((S, D), bf16), V((S, M), f32)],
        compiler_params=pltpu.CompilerParams(dimension_semantics=("arbitrary",),
                                             vmem_limit_bytes=120 * 2 ** 20),
    )(*args, B_w_o)
    return o[None]
```

```python
import numpy as np
import jax
import jax.numpy as jnp
from jax import lax
import jax.experimental.pallas as pl
import jax.experimental.pallas.tpu as pltpu

S, DA, H, D, M, DC = 2048, 448, 16, 256, 448, 1024
C = 128
NC = S // C
BQ = 256
f32, bf16 = jnp.float32, jnp.bfloat16
NT = (((1,), (1,)), ((), ()))


def _dft():
    n = np.arange(C)[None, :]
    f = np.arange(C)[:, None]
    ang = 2 * np.pi * f * n / (2 * C)
    fw = np.concatenate([np.cos(ang), -np.sin(ang)], 0)
    fw[C] = np.cos(np.pi * n[0])
    t = np.arange(2 * C)[:, None]
    fr = np.arange(C)[None, :]
    a2 = 2 * np.pi * t * fr / (2 * C)
    ic = 2 * np.cos(a2)
    ic[:, 0] = 1
    isn = -2 * np.sin(a2)
    isn[:, 0] = np.cos(np.pi * t[:, 0])
    inv = np.concatenate([ic, isn], 1) / (2 * C)
    inv2 = np.concatenate([inv[:C], inv[C:]], 1)
    return fw.astype(np.float32), inv2.astype(np.float32)


def _head(wref, hp, tr):
    w = wref[hp % 2]
    if tr:
        w = w.T
    lo = lax.bitcast_convert_type(w << 16, f32).astype(bf16)
    hi = lax.bitcast_convert_type(w & jnp.uint32(0xFFFF0000), f32).astype(bf16)
    return lo, hi


def _dot(a, b):
    return jnp.dot(a, b, preferred_element_type=f32)


def _kernel(aq, ak, av, sh, sk, sd, fw, inv, x, c, wq, wuk, wuv, wo, out,
            kvs, U, K, Z, cT, q_s, k_s, v_s, ctx_s, acc, wq_s, wk_s, wv_s, rq, rk, rv, sem):
    p = pl.program_id(0)

    def fetch(i):
        return [pltpu.make_async_copy(w.bitcast(jnp.uint32).at[:, i, :], r.at[i % 2], sem.at[n])
                for n, (w, r) in enumerate(((wq, rq), (wuk, rk), (wuv, rv)))]

    @pl.when(p == 0)
    def _():
        for cp in fetch(0):
            cp.start()
        cT[...] = c[...].T
        acc[...] = jnp.zeros_like(acc)
        Z[0] = jnp.zeros((DA, 2 * C), bf16)
        F = fw[...]
        lane = lax.broadcasted_iota(jnp.int32, (DA, C), 1)
        prev = jnp.zeros((DA, C), f32)
        for ch in range(NC):
            cs = slice(ch * C, (ch + 1) * C)
            cur = ak[:, cs].astype(f32)
            ks = jnp.zeros((DA, C), bf16)
            for j in (3, 2, 1, 0):
                kj = cur if j == 0 else pltpu.roll(jnp.where(lane >= C - j, prev, cur), j, 1)
                ks = ks + kj.astype(bf16) * sh[:, j:j + 1]
            prev = cur
            kv = ks * av[:, cs]
            kvs[ch] = kv
            U[ch] = _dot(kv, F)
            K[ch] = _dot(sk[:, cs], F)

    col0 = lax.broadcasted_iota(jnp.int32, (DA, C), 1) == 0
    for e in range(2):
        ch = 2 * p + e

        def body(d, carry):
            zr, zi = carry
            kr, ki = K[d, :, :C], K[d, :, C:]
            ur, ui = U[ch - d, :, :C], U[ch - d, :, C:]
            ii = ki * ui
            zr = zr + kr * ur - jnp.where(col0, 0.0, ii)
            zi = zi + jnp.where(col0, ii, kr * ui + ki * ur)
            return zr, zi
        z0 = jnp.zeros((DA, C), f32)
        zr, zi = lax.fori_loop(0, ch + 1, body, (z0, z0))
        Z[ch + 1, :, :C] = zr.astype(bf16)
        Z[ch + 1, :, C:] = zi.astype(bf16)
        y = (_dot(Z[ch + 1], inv[:2 * C, :]) + _dot(Z[ch], inv[2 * C:, :])).astype(bf16)
        r = pl.ds(pl.multiple_of(ch * C, C), C)
        y = y + kvs[ch] * sd[...]
        out[r, :DA] = (aq[:, r] * y).astype(f32).T.astype(bf16)

    for cp in fetch(p):
        cp.wait()

    @pl.when(p + 1 < H // 2)
    def _():
        for cp in fetch(p + 1):
            cp.start()

    for src, dst, tr in ((rq, wq_s, True), (rk, wk_s, False), (rv, wv_s, True)):
        dst[0], dst[1] = _head(src, p, tr)
    wqs, wks, wvs = wq_s, wk_s, wv_s
    tri = (lax.broadcasted_iota(jnp.int32, (BQ, BQ), 0) <= lax.broadcasted_iota(jnp.int32, (BQ, BQ), 1))
    for e in range(2):
        for t in range(0, S, 512):
            r = slice(t, t + 512)
            q_s[:, r] = (_dot(wqs[e], x[:, r]) * (D ** -0.5)).astype(bf16)
            k_s[r, :] = _dot(c[r, :], wks[e]).astype(bf16)
            v_s[:, r] = _dot(wvs[e], cT[:, r]).astype(bf16)
        for i in range(S // BQ):
            a, n = i * BQ, (i + 1) * BQ
            qi = q_s[:, a:n]
            s1 = jnp.where(tri, _dot(k_s[a:n, :], qi), -1e9)
            m = jnp.max(s1, 0, keepdims=True)
            if i:
                s0 = _dot(k_s[:a, :], qi)
                m = jnp.maximum(m, jnp.max(s0, 0, keepdims=True))
            p1 = jnp.exp(s1 - m)
            l = jnp.sum(p1, 0, keepdims=True)
            o = _dot(v_s[:, a:n], p1.astype(bf16))
            if i:
                p0 = jnp.exp(s0 - m)
                l = l + jnp.sum(p0, 0, keepdims=True)
                o = o + _dot(v_s[:, :a], p0.astype(bf16))
            ctx_s[:, a:n] = (o * (1.0 / l)).astype(bf16)
        for t in range(0, S, 512):
            r = slice(t, t + 512)
            acc[:, r] += _dot(wo[e], ctx_s[:, r])

    @pl.when(p == H // 2 - 1)
    def _():
        out[:, DA:] = acc[...].T.astype(bf16)


@jax.jit
def pallas_concat_heads__ssm_conv_h3__compressed_kv_cla__prompt_kernel(
        A_q, A_k, A_v, A_shift_k, A_ssm_k, A_ssm_D, B_x, B_c_kv, B_w_q, B_w_uk, B_w_uv, B_w_o):
    fw, inv = _dft()
    fw, inv = jnp.asarray(fw.T, bf16), jnp.asarray(inv.T, bf16)

    def full(a):
        nd = a.ndim
        return pl.BlockSpec(a.shape, lambda p: (0,) * nd, pipeline_mode=pl.Buffered(1))
    args = [A_q[0].T, A_k[0].T, A_v[0].T, A_shift_k, A_ssm_k, A_ssm_D[:, None], fw, inv,
            B_x[0].T, B_c_kv[0]]
    V = pltpu.VMEM
    o = pl.pallas_call(
        _kernel,
        grid=(H // 2,),
        in_specs=[full(a) for a in args] + [pl.BlockSpec(memory_space=pl.ANY)] * 3 + [pl.BlockSpec((2, M, D), lambda p: (p, 0, 0))],
        out_specs=pl.BlockSpec((S, DA + M), lambda p: (0, 0)),
        out_shape=jax.ShapeDtypeStruct((S, DA + M), bf16),
        scratch_shapes=[V((NC, DA, C), bf16), V((NC, DA, 2 * C), f32),
                        V((NC, DA, 2 * C), f32), V((NC + 1, DA, 2 * C), bf16), V((DC, S), bf16),
                        V((D, S), bf16), V((S, D), bf16), V((D, S), bf16),
                        V((D, S), bf16), V((M, S), f32),
                        V((2, D, M), bf16), V((2, DC, D), bf16), V((2, D, DC), bf16),
                        V((2, M, D), jnp.uint32), V((2, DC, D), jnp.uint32), V((2, DC, D), jnp.uint32),
                        pltpu.SemaphoreType.DMA((3,))],
        compiler_params=pltpu.CompilerParams(dimension_semantics=("arbitrary",),
                                             vmem_limit_bytes=120 * 2 ** 20),
    )(*args, B_w_q, B_w_uk, B_w_uv, B_w_o.transpose(0, 2, 1))
    return o[None]
```

```python
import numpy as np
import jax
import jax.numpy as jnp
from jax import lax
import jax.experimental.pallas as pl
import jax.experimental.pallas.tpu as pltpu

S, DA, H, D, M, DC = 2048, 448, 16, 256, 448, 1024
C = 128
NC = S // C
BQ = 256
f32, bf16 = jnp.float32, jnp.bfloat16
NT = (((1,), (1,)), ((), ()))


def _dft():
    n = np.arange(C)[None, :]
    f = np.arange(C)[:, None]
    ang = 2 * np.pi * f * n / (2 * C)
    fw = np.concatenate([np.cos(ang), -np.sin(ang)], 0)
    fw[C] = np.cos(np.pi * n[0])
    t = np.arange(2 * C)[:, None]
    fr = np.arange(C)[None, :]
    a2 = 2 * np.pi * t * fr / (2 * C)
    ic = 2 * np.cos(a2)
    ic[:, 0] = 1
    isn = -2 * np.sin(a2)
    isn[:, 0] = np.cos(np.pi * t[:, 0])
    inv = np.concatenate([ic, isn], 1) / (2 * C)
    inv2 = np.concatenate([inv[:C], inv[C:]], 1)
    return fw.astype(np.float32), inv2.astype(np.float32)


def _head(wref, hp, tr):
    w = wref[hp % 2]
    if tr:
        w = w.T
    lo = lax.bitcast_convert_type(w << 16, f32).astype(bf16)
    hi = lax.bitcast_convert_type(w & jnp.uint32(0xFFFF0000), f32).astype(bf16)
    return lo, hi


def _dot(a, b):
    return jnp.dot(a, b, preferred_element_type=f32)


def _kernel(aq, ak, av, sh, sk, sd, fw, inv, x, c, wq, wuk, wuv, wo, out,
            kvs, U, K, Z, cT, q_s, k_s, v_s, ctx_s, acc, wq_s, wk_s, wv_s, rq, rk, rv, sem):
    p = pl.program_id(0)

    def fetch(i):
        return [pltpu.make_async_copy(w.bitcast(jnp.uint32).at[:, i, :], r.at[i % 2], sem.at[n])
                for n, (w, r) in enumerate(((wq, rq), (wuk, rk), (wuv, rv)))]

    @pl.when(p == 0)
    def _():
        for cp in fetch(0):
            cp.start()
        cT[...] = c[...].T
        acc[...] = jnp.zeros_like(acc)
        Z[0] = jnp.zeros((DA, 2 * C), bf16)
        F = fw[...]
        lane = lax.broadcasted_iota(jnp.int32, (DA, C), 1)
        prev = jnp.zeros((DA, C), f32)
        for ch in range(NC):
            cs = slice(ch * C, (ch + 1) * C)
            cur = ak[:, cs].astype(f32)
            ks = jnp.zeros((DA, C), bf16)
            for j in (3, 2, 1, 0):
                kj = cur if j == 0 else pltpu.roll(jnp.where(lane >= C - j, prev, cur), j, 1)
                ks = ks + kj.astype(bf16) * sh[:, j:j + 1]
            prev = cur
            kv = ks * av[:, cs]
            kvs[ch] = kv
            U[ch] = _dot(kv, F)
            kf = _dot(sk[:, cs], F)
            K[ch, :, :C] = kf[:, :C]
            K[ch, :, C:2 * C] = jnp.where(lane == 0, 0.0, kf[:, C:])
            K[ch, :, 2 * C:] = jnp.where(lane == 0, kf[:, C:], kf[:, :C])

    def rows(g, _):
        rr = pl.ds(pl.multiple_of(g * 32, 32), 32)

        def mac(z, d, j):
            k0, k1, k2 = K[d, rr, :C], K[d, rr, C:2 * C], K[d, rr, 2 * C:]
            ur, ui = U[j, rr, :C], U[j, rr, C:]
            return z[0] + (k0 * ur - k1 * ui), z[1] + (k2 * ui + k1 * ur)

        def body(d, cr):
            return mac(cr[0], d, 2 * p - d), mac(cr[1], d, 2 * p + 1 - d)
        z0 = jnp.zeros((32, C), f32)
        zs = lax.fori_loop(0, 2 * p + 1, body, ((z0, z0), mac((z0, z0), 2 * p + 1, 0)))
        for e in range(2):
            Z[2 * p + e + 1, rr, :C] = zs[e][0].astype(bf16)
            Z[2 * p + e + 1, rr, C:] = zs[e][1].astype(bf16)
        return 0
    lax.fori_loop(0, DA // 32, rows, 0)
    for e in range(2):
        ch = 2 * p + e
        y = (_dot(Z[ch + 1], inv[:2 * C, :]) + _dot(Z[ch], inv[2 * C:, :])).astype(bf16)
        r = pl.ds(pl.multiple_of(ch * C, C), C)
        y = y + kvs[ch] * sd[...]
        out[r, :DA] = (aq[:, r] * y).astype(f32).T.astype(bf16)

    for cp in fetch(p):
        cp.wait()

    @pl.when(p + 1 < H // 2)
    def _():
        for cp in fetch(p + 1):
            cp.start()

    for src, dst, tr in ((rq, wq_s, True), (rk, wk_s, False), (rv, wv_s, True)):
        dst[0], dst[1] = _head(src, p, tr)
    wqs, wks, wvs = wq_s, wk_s, wv_s
    tri = (lax.broadcasted_iota(jnp.int32, (BQ, BQ), 0) <= lax.broadcasted_iota(jnp.int32, (BQ, BQ), 1))
    @pl.loop(0, 2)
    def _(e):
        for t in range(0, S, 512):
            r = slice(t, t + 512)
            q_s[:, r] = (_dot(wqs[e], x[:, r]) * (D ** -0.5)).astype(bf16)
            k_s[r, :] = _dot(c[r, :], wks[e]).astype(bf16)
            v_s[:, r] = _dot(wvs[e], cT[:, r]).astype(bf16)
        def qk(i):
            a, n = i * BQ, (i + 1) * BQ
            qi = q_s[:, a:n]
            s1 = jnp.where(tri, _dot(k_s[a:n, :], qi), -1e9)
            m = jnp.max(s1, 0, keepdims=True)
            s0 = None
            if i:
                s0 = _dot(k_s[:a, :], qi)
                m = jnp.maximum(m, jnp.max(s0, 0, keepdims=True))
            return s0, s1, m
        nxt = qk(0)
        for i in range(S // BQ):
            a, n = i * BQ, (i + 1) * BQ
            s0, s1, m = nxt
            if n < S:
                nxt = qk(i + 1)
            p1 = jnp.exp(s1 - m)
            l = jnp.sum(p1, 0, keepdims=True)
            o = _dot(v_s[:, a:n], p1.astype(bf16))
            if i:
                p0 = jnp.exp(s0 - m)
                l = l + jnp.sum(p0, 0, keepdims=True)
                o = o + _dot(v_s[:, :a], p0.astype(bf16))
            ctx_s[:, a:n] = (o * (1.0 / l)).astype(bf16)
        for t in range(0, S, 512):
            r = slice(t, t + 512)
            acc[:, r] += _dot(wo[e], ctx_s[:, r])

    @pl.when(p == H // 2 - 1)
    def _():
        out[:, DA:] = acc[...].T.astype(bf16)


@jax.jit
def pallas_concat_heads__ssm_conv_h3__compressed_kv_cla__prompt_kernel(
        A_q, A_k, A_v, A_shift_k, A_ssm_k, A_ssm_D, B_x, B_c_kv, B_w_q, B_w_uk, B_w_uv, B_w_o):
    fw, inv = _dft()
    fw, inv = jnp.asarray(fw.T, bf16), jnp.asarray(inv.T, bf16)

    def full(a):
        nd = a.ndim
        return pl.BlockSpec(a.shape, lambda p: (0,) * nd, pipeline_mode=pl.Buffered(1))
    args = [A_q[0].T, A_k[0].T, A_v[0].T, A_shift_k, A_ssm_k, A_ssm_D[:, None], fw, inv,
            B_x[0].T, B_c_kv[0]]
    V = pltpu.VMEM
    o = pl.pallas_call(
        _kernel,
        grid=(H // 2,),
        in_specs=[full(a) for a in args] + [pl.BlockSpec(memory_space=pl.ANY)] * 3 + [pl.BlockSpec((2, M, D), lambda p: (p, 0, 0))],
        out_specs=pl.BlockSpec((S, DA + M), lambda p: (0, 0)),
        out_shape=jax.ShapeDtypeStruct((S, DA + M), bf16),
        scratch_shapes=[V((NC, DA, C), bf16), V((NC, DA, 2 * C), f32),
                        V((NC, DA, 3 * C), f32), V((NC + 1, DA, 2 * C), bf16), V((DC, S), bf16),
                        V((D, S), bf16), V((S, D), bf16), V((D, S), bf16),
                        V((D, S), bf16), V((M, S), f32),
                        V((2, D, M), bf16), V((2, DC, D), bf16), V((2, D, DC), bf16),
                        V((2, M, D), jnp.uint32), V((2, DC, D), jnp.uint32), V((2, DC, D), jnp.uint32),
                        pltpu.SemaphoreType.DMA((3,))],
        compiler_params=pltpu.CompilerParams(dimension_semantics=("arbitrary",),
                                             vmem_limit_bytes=120 * 2 ** 20),
    )(*args, B_w_q, B_w_uk, B_w_uv, B_w_o.transpose(0, 2, 1))
    return o[None]
```

```python
import numpy as np
import jax
import jax.numpy as jnp
from jax import lax
import jax.experimental.pallas as pl
import jax.experimental.pallas.tpu as pltpu

S, DA, H, D, M, DC = 2048, 448, 16, 256, 448, 1024
C = 128
NC = S // C
BQ = 256
f32, bf16 = jnp.float32, jnp.bfloat16
NT = (((1,), (1,)), ((), ()))


def _dft():
    n = np.arange(C)[None, :]
    f = np.arange(C)[:, None]
    ang = 2 * np.pi * f * n / (2 * C)
    fw = np.concatenate([np.cos(ang), -np.sin(ang)], 0)
    fw[C] = np.cos(np.pi * n[0])
    t = np.arange(2 * C)[:, None]
    fr = np.arange(C)[None, :]
    a2 = 2 * np.pi * t * fr / (2 * C)
    ic = 2 * np.cos(a2)
    ic[:, 0] = 1
    isn = -2 * np.sin(a2)
    isn[:, 0] = np.cos(np.pi * t[:, 0])
    inv = np.concatenate([ic, isn], 1) / (2 * C)
    inv2 = np.concatenate([inv[:C], inv[C:]], 1)
    return fw.astype(np.float32), inv2.astype(np.float32)


def _head(wref, hp, tr):
    w = wref[hp % 2]
    if tr:
        w = w.T
    lo = lax.bitcast_convert_type(w << 16, f32).astype(bf16)
    hi = lax.bitcast_convert_type(w & jnp.uint32(0xFFFF0000), f32).astype(bf16)
    return lo, hi


def _dot(a, b):
    return jnp.dot(a, b, preferred_element_type=f32)


def _kernel(aq, ak, av, sh, sk, sd, fw, inv, x, c, wq, wuk, wuv, wo, out,
            kvs, U, K, Z, cT, q_s, k_s, v_s, ctx_s, acc, wq_s, wk_s, wv_s, rq, rk, rv, sem):
    p = pl.program_id(0)

    def fetch(i):
        return [pltpu.make_async_copy(w.bitcast(jnp.uint32).at[:, i, :], r.at[i % 2], sem.at[n])
                for n, (w, r) in enumerate(((wq, rq), (wuk, rk), (wuv, rv)))]

    @pl.when(p == 0)
    def _():
        for cp in fetch(0):
            cp.start()
        Z[0] = jnp.zeros((DA, 2 * C), bf16)
        F = fw[...]
        lane = lax.broadcasted_iota(jnp.int32, (DA, C), 1)

        @pl.loop(0, NC)
        def _(ch):
            cs = pl.ds(pl.multiple_of(ch * C, C), C)
            cT[:, cs] = c[cs, :].T
            acc[:, cs] = jnp.zeros((M, C), f32)
            prev = ak[:, pl.ds(pl.multiple_of(jnp.maximum(ch - 1, 0) * C, C), C)].astype(f32)
            prev = jnp.where(ch > 0, prev, 0.0)
            cur = ak[:, cs].astype(f32)
            ks = jnp.zeros((DA, C), bf16)
            for j in (3, 2, 1, 0):
                kj = cur if j == 0 else pltpu.roll(jnp.where(lane >= C - j, prev, cur), j, 1)
                ks = ks + kj.astype(bf16) * sh[:, j:j + 1]
            kv = ks * av[:, cs]
            kvs[ch] = kv
            U[ch] = _dot(kv, F)
            kf = _dot(sk[:, cs], F)
            K[ch, :, :C] = kf[:, :C]
            K[ch, :, C:2 * C] = jnp.where(lane == 0, 0.0, kf[:, C:])
            K[ch, :, 2 * C:] = jnp.where(lane == 0, kf[:, C:], kf[:, :C])

    def rows(g, _):
        rr = pl.ds(pl.multiple_of(g * 64, 64), 64)

        def mac(z, d, j):
            k0, k1, k2 = K[d, rr, :C], K[d, rr, C:2 * C], K[d, rr, 2 * C:]
            ur, ui = U[j, rr, :C], U[j, rr, C:]
            return z[0] + (k0 * ur - k1 * ui), z[1] + (k2 * ui + k1 * ur)

        def body(d, cr):
            return mac(cr[0], d, 2 * p - d), mac(cr[1], d, 2 * p + 1 - d)
        z0 = jnp.zeros((64, C), f32)
        zs = lax.fori_loop(0, 2 * p + 1, body, ((z0, z0), mac((z0, z0), 2 * p + 1, 0)))
        for e in range(2):
            Z[2 * p + e + 1, rr, :C] = zs[e][0].astype(bf16)
            Z[2 * p + e + 1, rr, C:] = zs[e][1].astype(bf16)
        return 0
    lax.fori_loop(0, DA // 64, rows, 0)
    for e in range(2):
        ch = 2 * p + e
        y = (_dot(Z[ch + 1], inv[:2 * C, :]) + _dot(Z[ch], inv[2 * C:, :])).astype(bf16)
        r = pl.ds(pl.multiple_of(ch * C, C), C)
        y = y + kvs[ch] * sd[...]
        out[r, :DA] = (aq[:, r] * y).astype(f32).T.astype(bf16)

    for cp in fetch(p):
        cp.wait()

    @pl.when(p + 1 < H // 2)
    def _():
        for cp in fetch(p + 1):
            cp.start()

    for src, dst, tr in ((rq, wq_s, True), (rk, wk_s, False), (rv, wv_s, True)):
        dst[0], dst[1] = _head(src, p, tr)
    wqs, wks, wvs = wq_s, wk_s, wv_s
    tri = (lax.broadcasted_iota(jnp.int32, (BQ, BQ), 0) <= lax.broadcasted_iota(jnp.int32, (BQ, BQ), 1))
    @pl.loop(0, 2)
    def _(e):
        for t in range(0, S, 512):
            r = slice(t, t + 512)
            q_s[:, r] = (_dot(wqs[e], x[:, r]) * (D ** -0.5)).astype(bf16)
            k_s[r, :] = _dot(c[r, :], wks[e]).astype(bf16)
            v_s[:, r] = _dot(wvs[e], cT[:, r]).astype(bf16)
        def qk(i):
            a, n = i * BQ, (i + 1) * BQ
            qi = q_s[:, a:n]
            s1 = jnp.where(tri, _dot(k_s[a:n, :], qi), -1e9)
            m = jnp.max(s1, 0, keepdims=True)
            s0 = None
            if i:
                s0 = _dot(k_s[:a, :], qi)
                m = jnp.maximum(m, jnp.max(s0, 0, keepdims=True))
            return s0, s1, m
        nxt = qk(0)
        for i in range(S // BQ):
            a, n = i * BQ, (i + 1) * BQ
            s0, s1, m = nxt
            if n < S:
                nxt = qk(i + 1)
            p1 = jnp.exp(s1 - m)
            l = jnp.sum(p1, 0, keepdims=True)
            o = _dot(v_s[:, a:n], p1.astype(bf16))
            if i:
                p0 = jnp.exp(s0 - m)
                l = l + jnp.sum(p0, 0, keepdims=True)
                o = o + _dot(v_s[:, :a], p0.astype(bf16))
            ctx_s[:, a:n] = (o * (1.0 / l)).astype(bf16)
        for t in range(0, S, 512):
            r = slice(t, t + 512)
            acc[:, r] += _dot(wo[e], ctx_s[:, r])

    @pl.when(p == H // 2 - 1)
    def _():
        @pl.loop(0, S // 256)
        def _(t):
            r = pl.ds(pl.multiple_of(t * 256, 256), 256)
            out[r, DA:] = acc[:, r].T.astype(bf16)


@jax.jit
def pallas_concat_heads__ssm_conv_h3__compressed_kv_cla__prompt_kernel(
        A_q, A_k, A_v, A_shift_k, A_ssm_k, A_ssm_D, B_x, B_c_kv, B_w_q, B_w_uk, B_w_uv, B_w_o):
    fw, inv = _dft()
    fw, inv = jnp.asarray(fw.T, bf16), jnp.asarray(inv.T, bf16)

    def full(a):
        nd = a.ndim
        return pl.BlockSpec(a.shape, lambda p: (0,) * nd, pipeline_mode=pl.Buffered(1))
    args = [A_q[0].T, A_k[0].T, A_v[0].T, A_shift_k, A_ssm_k, A_ssm_D[:, None], fw, inv,
            B_x[0].T, B_c_kv[0]]
    V = pltpu.VMEM
    o = pl.pallas_call(
        _kernel,
        grid=(H // 2,),
        in_specs=[full(a) for a in args] + [pl.BlockSpec(memory_space=pl.ANY)] * 3 + [pl.BlockSpec((2, M, D), lambda p: (p, 0, 0))],
        out_specs=pl.BlockSpec((S, DA + M), lambda p: (0, 0)),
        out_shape=jax.ShapeDtypeStruct((S, DA + M), bf16),
        scratch_shapes=[V((NC, DA, C), bf16), V((NC, DA, 2 * C), f32),
                        V((NC, DA, 3 * C), f32), V((NC + 1, DA, 2 * C), bf16), V((DC, S), bf16),
                        V((D, S), bf16), V((S, D), bf16), V((D, S), bf16),
                        V((D, S), bf16), V((M, S), f32),
                        V((2, D, M), bf16), V((2, DC, D), bf16), V((2, D, DC), bf16),
                        V((2, M, D), jnp.uint32), V((2, DC, D), jnp.uint32), V((2, DC, D), jnp.uint32),
                        pltpu.SemaphoreType.DMA((3,))],
        compiler_params=pltpu.CompilerParams(dimension_semantics=("arbitrary",),
                                             flags={"XLA_TPU_FORCE_LP_LLO_SCHEDULER": True}, vmem_limit_bytes=120 * 2 ** 20),
    )(*args, B_w_q, B_w_uk, B_w_uv, B_w_o.transpose(0, 2, 1))
    return o[None]
```

```python
import numpy as np
import jax
import jax.numpy as jnp
from jax import lax
import jax.experimental.pallas as pl
import jax.experimental.pallas.tpu as pltpu

S, DA, H, D, M, DC = 2048, 448, 16, 256, 448, 1024
C = 128
NC = S // C
BQ = 256
f32, bf16 = jnp.float32, jnp.bfloat16
NT = (((1,), (1,)), ((), ()))


def _dft():
    n = np.arange(C)[None, :]
    f = np.arange(C)[:, None]
    ang = 2 * np.pi * f * n / (2 * C)
    fw = np.concatenate([np.cos(ang), -np.sin(ang)], 0)
    fw[C] = np.cos(np.pi * n[0])
    t = np.arange(2 * C)[:, None]
    fr = np.arange(C)[None, :]
    a2 = 2 * np.pi * t * fr / (2 * C)
    ic = 2 * np.cos(a2)
    ic[:, 0] = 1
    isn = -2 * np.sin(a2)
    isn[:, 0] = np.cos(np.pi * t[:, 0])
    inv = np.concatenate([ic, isn], 1) / (2 * C)
    inv2 = np.concatenate([inv[:C], inv[C:]], 1)
    return fw.astype(np.float32), inv2.astype(np.float32)


def _head(wref, hp, tr):
    w = wref[hp % 2]
    if tr:
        w = w.T
    lo = lax.bitcast_convert_type(w << 16, f32).astype(bf16)
    hi = lax.bitcast_convert_type(w & jnp.uint32(0xFFFF0000), f32).astype(bf16)
    return lo, hi


def _dot(a, b):
    return jnp.dot(a, b, preferred_element_type=f32)


def _kernel(aq, ak, av, sh, sk, sd, fw, inv, x, c, wq, wuk, wuv, wo, out,
            kvs, U, K, Z, cT, q_s, k_s, v_s, ctx_s, acc, wq_s, wk_s, wv_s, rq, rk, rv, sem):
    p = pl.program_id(0)

    def fetch(i):
        return [pltpu.make_async_copy(w.bitcast(jnp.uint32).at[:, i, :], r.at[i % 2], sem.at[n])
                for n, (w, r) in enumerate(((wq, rq), (wuk, rk), (wuv, rv)))]

    @pl.when(p == 0)
    def _():
        for cp in fetch(0):
            cp.start()
        Z[0] = jnp.zeros((DA, 2 * C), bf16)
        F = fw[...]
        lane = lax.broadcasted_iota(jnp.int32, (DA, C), 1)

        @pl.loop(0, NC)
        def _(ch):
            cs = pl.ds(pl.multiple_of(ch * C, C), C)
            cT[:, cs] = c[cs, :].T
            acc[:, cs] = jnp.zeros((M, C), f32)
            prev = ak[:, pl.ds(pl.multiple_of(jnp.maximum(ch - 1, 0) * C, C), C)].astype(f32)
            prev = jnp.where(ch > 0, prev, 0.0)
            cur = ak[:, cs].astype(f32)
            ks = jnp.zeros((DA, C), bf16)
            for j in (3, 2, 1, 0):
                kj = cur if j == 0 else pltpu.roll(jnp.where(lane >= C - j, prev, cur), j, 1)
                ks = ks + kj.astype(bf16) * sh[:, j:j + 1]
            kv = ks * av[:, cs]
            kvs[ch] = kv
            U[ch] = _dot(kv, F)
            kf = _dot(sk[:, cs], F)
            K[ch, :, :C] = kf[:, :C]
            K[ch, :, C:2 * C] = jnp.where(lane == 0, 0.0, kf[:, C:])
            K[ch, :, 2 * C:] = jnp.where(lane == 0, kf[:, C:], kf[:, :C])

    def mac(e, g):
        rr = pl.ds(pl.multiple_of(e * (DA // 2) + g * 16, 16), 16)
        zr = zi = ar = ai = jnp.zeros((16, C), f32)
        for t in range(NC + 1):
            first = t <= p
            d = jnp.where(first, t, t - p - 1)
            j = jnp.where(first, p - t, NC - t)
            k0, k1, k2 = K[d, rr, :C], K[d, rr, C:2 * C], K[d, rr, 2 * C:]
            ur, ui = U[j, rr, :C], U[j, rr, C:]
            tr, ti = k0 * ur - k1 * ui, k2 * ui + k1 * ur
            if 0 < t <= NC // 2:
                ar, ai = jnp.where(t == p + 1, zr, ar), jnp.where(t == p + 1, zi, ai)
                zr, zi = jnp.where(t == p + 1, 0.0, zr), jnp.where(t == p + 1, 0.0, zi)
            zr, zi = zr + tr, zi + ti
        Z[p + 1, rr, :C], Z[p + 1, rr, C:] = ar.astype(bf16), ai.astype(bf16)
        Z[NC - p, rr, :C], Z[NC - p, rr, C:] = zr.astype(bf16), zi.astype(bf16)

    for cp in fetch(p):
        cp.wait()

    @pl.when(p + 1 < H // 2)
    def _():
        for cp in fetch(p + 1):
            cp.start()

    for src, dst, tr in ((rq, wq_s, True), (rk, wk_s, False), (rv, wv_s, True)):
        dst[0], dst[1] = _head(src, p, tr)
    wqs, wks, wvs = wq_s, wk_s, wv_s
    tri = (lax.broadcasted_iota(jnp.int32, (BQ, BQ), 0) <= lax.broadcasted_iota(jnp.int32, (BQ, BQ), 1))
    @pl.loop(0, 2)
    def _(e):
        for t in range(0, S, 512):
            r = slice(t, t + 512)
            q_s[:, r] = (_dot(wqs[e], x[:, r]) * (D ** -0.5)).astype(bf16)
            k_s[r, :] = _dot(c[r, :], wks[e]).astype(bf16)
            v_s[:, r] = _dot(wvs[e], cT[:, r]).astype(bf16)
            for g in range(t // 128, min(t // 128 + 4, DA // 32)):
                mac(e, g)
        def qk(i):
            a, n = i * BQ, (i + 1) * BQ
            qi = q_s[:, a:n]
            s1 = jnp.where(tri, _dot(k_s[a:n, :], qi), -1e9)
            m = jnp.max(s1, 0, keepdims=True)
            s0 = None
            if i:
                s0 = _dot(k_s[:a, :], qi)
                m = jnp.maximum(m, jnp.max(s0, 0, keepdims=True))
            return s0, s1, m
        nxt = qk(0)
        for i in range(S // BQ):
            a, n = i * BQ, (i + 1) * BQ
            s0, s1, m = nxt
            if n < S:
                nxt = qk(i + 1)
            p1 = jnp.exp(s1 - m)
            l = jnp.sum(p1, 0, keepdims=True)
            o = _dot(v_s[:, a:n], p1.astype(bf16))
            if i:
                p0 = jnp.exp(s0 - m)
                l = l + jnp.sum(p0, 0, keepdims=True)
                o = o + _dot(v_s[:, :a], p0.astype(bf16))
            ctx_s[:, a:n] = (o * (1.0 / l)).astype(bf16)
        for t in range(0, S, 512):
            r = slice(t, t + 512)
            acc[:, r] += _dot(wo[e], ctx_s[:, r])

    @pl.when(p == H // 2 - 1)
    def _():
        @pl.loop(0, S // 256)
        def _(t):
            r = pl.ds(pl.multiple_of(t * 256, 256), 256)
            out[r, DA:] = acc[:, r].T.astype(bf16)
            for u in range(2):
                ch = 2 * t + u
                y = (_dot(Z[ch + 1], inv[:2 * C, :]) + _dot(Z[ch], inv[2 * C:, :])).astype(bf16)
                rc = pl.ds(pl.multiple_of(ch * C, C), C)
                y = y + kvs[ch] * sd[...]
                out[rc, :DA] = (aq[:, rc] * y).astype(f32).T.astype(bf16)


@jax.jit
def pallas_concat_heads__ssm_conv_h3__compressed_kv_cla__prompt_kernel(
        A_q, A_k, A_v, A_shift_k, A_ssm_k, A_ssm_D, B_x, B_c_kv, B_w_q, B_w_uk, B_w_uv, B_w_o):
    fw, inv = _dft()
    fw, inv = jnp.asarray(fw.T, bf16), jnp.asarray(inv.T, bf16)

    def full(a):
        nd = a.ndim
        return pl.BlockSpec(a.shape, lambda p: (0,) * nd, pipeline_mode=pl.Buffered(1))
    args = [A_q[0].T, A_k[0].T, A_v[0].T, A_shift_k, A_ssm_k, A_ssm_D[:, None], fw, inv,
            B_x[0].T, B_c_kv[0]]
    V = pltpu.VMEM
    o = pl.pallas_call(
        _kernel,
        grid=(H // 2,),
        in_specs=[full(a) for a in args] + [pl.BlockSpec(memory_space=pl.ANY)] * 3 + [pl.BlockSpec((2, M, D), lambda p: (p, 0, 0))],
        out_specs=pl.BlockSpec((S, DA + M), lambda p: (0, 0)),
        out_shape=jax.ShapeDtypeStruct((S, DA + M), bf16),
        scratch_shapes=[V((NC, DA, C), bf16), V((NC, DA, 2 * C), f32),
                        V((NC, DA, 3 * C), f32), V((NC + 1, DA, 2 * C), bf16), V((DC, S), bf16),
                        V((D, S), bf16), V((S, D), bf16), V((D, S), bf16),
                        V((D, S), bf16), V((M, S), f32),
                        V((2, D, M), bf16), V((2, DC, D), bf16), V((2, D, DC), bf16),
                        V((2, M, D), jnp.uint32), V((2, DC, D), jnp.uint32), V((2, DC, D), jnp.uint32),
                        pltpu.SemaphoreType.DMA((3,))],
        compiler_params=pltpu.CompilerParams(dimension_semantics=("arbitrary",),
                                             flags={"XLA_TPU_FORCE_LP_LLO_SCHEDULER": False}, vmem_limit_bytes=120 * 2 ** 20),
    )(*args, B_w_q, B_w_uk, B_w_uv, B_w_o.transpose(0, 2, 1))
    return o[None]
```

```python
import numpy as np
import jax
import jax.numpy as jnp
from jax import lax
import jax.experimental.pallas as pl
import jax.experimental.pallas.tpu as pltpu

S, DA, H, D, M, DC = 2048, 448, 16, 256, 448, 1024
C = 128
NC = S // C
BQ = 256
f32, bf16 = jnp.float32, jnp.bfloat16
NT = (((1,), (1,)), ((), ()))


def _dft():
    n = np.arange(C)[None, :]
    f = np.arange(C)[:, None]
    ang = 2 * np.pi * f * n / (2 * C)
    fw = np.concatenate([np.cos(ang), -np.sin(ang)], 0)
    fw[C] = np.cos(np.pi * n[0])
    t = np.arange(2 * C)[:, None]
    fr = np.arange(C)[None, :]
    a2 = 2 * np.pi * t * fr / (2 * C)
    ic = 2 * np.cos(a2)
    ic[:, 0] = 1
    isn = -2 * np.sin(a2)
    isn[:, 0] = np.cos(np.pi * t[:, 0])
    inv = np.concatenate([ic, isn], 1) / (2 * C)
    inv2 = np.concatenate([inv[:C], inv[C:]], 1)
    return fw.astype(np.float32), inv2.astype(np.float32)


def _head(wref, hp, tr):
    w = wref[hp % 2]
    if tr:
        w = w.T
    lo = lax.bitcast_convert_type(w << 16, f32).astype(bf16)
    hi = lax.bitcast_convert_type(w & jnp.uint32(0xFFFF0000), f32).astype(bf16)
    return lo, hi


def _dot(a, b):
    return jnp.dot(a, b, preferred_element_type=f32)


def _kernel(aq_h, ak_h, av_h, sh, sk_h, sd, fw, inv, x, c, wq, wuk, wuv, wo, out,
            kvs, U, K, Z, cT, q_s, k_s, v_s, ctx_s, acc, wq_s, wk_s, wv_s, rq, rk, rv, sem, aq, ak, av, sk, sem2):
    p = pl.program_id(0)

    def fetch(i):
        return [pltpu.make_async_copy(w.bitcast(jnp.uint32).at[:, i, :], r.at[i % 2], sem.at[n])
                for n, (w, r) in enumerate(((wq, rq), (wuk, rk), (wuv, rv)))]

    a_in = [pltpu.make_async_copy(h_, v_, sem2.at[n])
            for n, (h_, v_) in enumerate(((aq_h, aq), (ak_h, ak), (av_h, av), (sk_h, sk)))]

    @pl.when(p == 0)
    def _():
        for cp in fetch(0):
            cp.start()
        for cp in a_in:
            cp.start()

        @pl.loop(0, NC)
        def _(ch):
            cs = pl.ds(pl.multiple_of(ch * C, C), C)
            cT[:, cs] = c[cs, :].T
            acc[:, cs] = jnp.zeros((M, C), f32)

    for cp in fetch(p):
        cp.wait()

    @pl.when(p + 1 < H // 2)
    def _():
        for cp in fetch(p + 1):
            cp.start()

    for src, dst, tr in ((rq, wq_s, True), (rk, wk_s, False), (rv, wv_s, True)):
        dst[0], dst[1] = _head(src, p, tr)
    wqs, wks, wvs = wq_s, wk_s, wv_s
    tri = (lax.broadcasted_iota(jnp.int32, (BQ, BQ), 0) <= lax.broadcasted_iota(jnp.int32, (BQ, BQ), 1))
    @pl.loop(0, 2)
    def _(e):
        for t in range(0, S, 512):
            r = slice(t, t + 512)
            q_s[:, r] = (_dot(wqs[e], x[:, r]) * (D ** -0.5)).astype(bf16)
            k_s[r, :] = _dot(c[r, :], wks[e]).astype(bf16)
            v_s[:, r] = _dot(wvs[e], cT[:, r]).astype(bf16)
        def qk(i):
            a, n = i * BQ, (i + 1) * BQ
            qi = q_s[:, a:n]
            s1 = jnp.where(tri, _dot(k_s[a:n, :], qi), -1e9)
            m = jnp.max(s1, 0, keepdims=True)
            s0 = None
            if i:
                s0 = _dot(k_s[:a, :], qi)
                m = jnp.maximum(m, jnp.max(s0, 0, keepdims=True))
            return s0, s1, m
        nxt = qk(0)
        for i in range(S // BQ):
            a, n = i * BQ, (i + 1) * BQ
            s0, s1, m = nxt
            if n < S:
                nxt = qk(i + 1)
            p1 = jnp.exp(s1 - m)
            l = jnp.sum(p1, 0, keepdims=True)
            o = _dot(v_s[:, a:n], p1.astype(bf16))
            if i:
                p0 = jnp.exp(s0 - m)
                l = l + jnp.sum(p0, 0, keepdims=True)
                o = o + _dot(v_s[:, :a], p0.astype(bf16))
            ctx_s[:, a:n] = (o * (1.0 / l)).astype(bf16)
        for t in range(0, S, 512):
            r = slice(t, t + 512)
            acc[:, r] += _dot(wo[e], ctx_s[:, r])

    @pl.when(p == H // 2 - 1)
    def _():
        for cp in a_in:
            cp.wait()
        Z[0] = jnp.zeros((DA, 2 * C), bf16)
        F = fw[...]
        lane = lax.broadcasted_iota(jnp.int32, (DA, C), 1)

        @pl.loop(0, NC)
        def _(ch):
            cs = pl.ds(pl.multiple_of(ch * C, C), C)
            prev = ak[:, pl.ds(pl.multiple_of(jnp.maximum(ch - 1, 0) * C, C), C)].astype(f32)
            prev = jnp.where(ch > 0, prev, 0.0)
            cur = ak[:, cs].astype(f32)
            ks = jnp.zeros((DA, C), bf16)
            for j in (3, 2, 1, 0):
                kj = cur if j == 0 else pltpu.roll(jnp.where(lane >= C - j, prev, cur), j, 1)
                ks = ks + kj.astype(bf16) * sh[:, j:j + 1]
            kv = ks * av[:, cs]
            kvs[ch] = kv
            U[ch] = _dot(kv, F)
            kf = _dot(sk[:, cs], F)
            K[ch, :, :C] = kf[:, :C]
            K[ch, :, C:2 * C] = jnp.where(lane == 0, 0.0, kf[:, C:])
            K[ch, :, 2 * C:] = jnp.where(lane == 0, kf[:, C:], kf[:, :C])

        @pl.loop(0, DA // 16)
        def _(g):
            res = []
            for hf in range(2):
                rr = pl.ds(pl.multiple_of(g * 16 + hf * 8, 8), 8)
                zs = []
                for c0 in range(0, NC, 4):
                    z = [None] * 4
                    for j0 in range(0, c0 + 1, 4):
                        u = [(U[j, rr, :C], U[j, rr, C:]) for j in range(j0, j0 + 4)]
                        for d in range(max(c0 - j0 - 3, 0), c0 - j0 + 4):
                            k0, k1, k2 = K[d, rr, :C], K[d, rr, C:2 * C], K[d, rr, 2 * C:]
                            for i in range(4):
                                j = c0 + i - d - j0
                                if 0 <= j < 4:
                                    ur, ui = u[j]
                                    t = (k0 * ur - k1 * ui, k2 * ui + k1 * ur)
                                    z[i] = t if z[i] is None else (z[i][0] + t[0], z[i][1] + t[1])
                    zs += z
                res.append(zs)
            r16 = pl.ds(pl.multiple_of(g * 16, 16), 16)
            for ch in range(NC):
                for h in range(2):
                    Z[ch + 1, r16, h * C:(h + 1) * C] = jnp.concatenate(
                        [res[0][ch][h], res[1][ch][h]], 0).astype(bf16)

        @pl.loop(0, S // 256)
        def _(t):
            r = pl.ds(pl.multiple_of(t * 256, 256), 256)
            out[r, DA:] = acc[:, r].T.astype(bf16)
            for u in range(2):
                ch = 2 * t + u
                y = (_dot(Z[ch + 1], inv[:2 * C, :]) + _dot(Z[ch], inv[2 * C:, :])).astype(bf16)
                rc = pl.ds(pl.multiple_of(ch * C, C), C)
                y = y + kvs[ch] * sd[...]
                out[rc, :DA] = (aq[:, rc] * y).astype(f32).T.astype(bf16)


@jax.jit
def pallas_concat_heads__ssm_conv_h3__compressed_kv_cla__prompt_kernel(
        A_q, A_k, A_v, A_shift_k, A_ssm_k, A_ssm_D, B_x, B_c_kv, B_w_q, B_w_uk, B_w_uv, B_w_o):
    fw, inv = _dft()
    fw, inv = jnp.asarray(fw.T, bf16), jnp.asarray(inv.T, bf16)

    def full(a):
        nd = a.ndim
        return pl.BlockSpec(a.shape, lambda p: (0,) * nd, pipeline_mode=pl.Buffered(1))
    args = [A_q[0].T, A_k[0].T, A_v[0].T, A_shift_k, A_ssm_k, A_ssm_D[:, None], fw, inv,
            B_x[0].T, B_c_kv[0]]
    V = pltpu.VMEM
    o = pl.pallas_call(
        _kernel,
        grid=(H // 2,),
        in_specs=[pl.BlockSpec(memory_space=pl.ANY) if n in (0, 1, 2, 4) else full(a)
                  for n, a in enumerate(args)] + [pl.BlockSpec(memory_space=pl.ANY)] * 3 + [pl.BlockSpec((2, M, D), lambda p: (p, 0, 0))],
        out_specs=pl.BlockSpec((S, DA + M), lambda p: (0, 0)),
        out_shape=jax.ShapeDtypeStruct((S, DA + M), bf16),
        scratch_shapes=[V((NC, DA, C), bf16), V((NC, DA, 2 * C), f32),
                        V((NC, DA, 3 * C), f32), V((NC + 1, DA, 2 * C), bf16), V((DC, S), bf16),
                        V((D, S), bf16), V((S, D), bf16), V((D, S), bf16),
                        V((D, S), bf16), V((M, S), f32),
                        V((2, D, M), bf16), V((2, DC, D), bf16), V((2, D, DC), bf16),
                        V((2, M, D), jnp.uint32), V((2, DC, D), jnp.uint32), V((2, DC, D), jnp.uint32),
                        pltpu.SemaphoreType.DMA((3,))] + [V((DA, S), bf16)] * 4 + [pltpu.SemaphoreType.DMA((4,))],
        compiler_params=pltpu.CompilerParams(dimension_semantics=("arbitrary",),
                                             flags={"XLA_TPU_FORCE_LP_LLO_SCHEDULER": False}, vmem_limit_bytes=120 * 2 ** 20),
    )(*args, B_w_q, B_w_uk, B_w_uv, B_w_o.transpose(0, 2, 1))
    return o[None]
```

```python
import numpy as np
import jax
import jax.numpy as jnp
from jax import lax
import jax.experimental.pallas as pl
import jax.experimental.pallas.tpu as pltpu

S, DA, H, D, M, DC = 2048, 448, 16, 256, 448, 1024
C = 128
NC = S // C
BQ = 256
f32, bf16 = jnp.float32, jnp.bfloat16
NT = (((1,), (1,)), ((), ()))


def _dft():
    n = np.arange(C)[None, :]
    f = np.arange(C)[:, None]
    ang = 2 * np.pi * f * n / (2 * C)
    fw = np.concatenate([np.cos(ang), -np.sin(ang)], 0)
    fw[C] = np.cos(np.pi * n[0])
    t = np.arange(2 * C)[:, None]
    fr = np.arange(C)[None, :]
    a2 = 2 * np.pi * t * fr / (2 * C)
    ic = 2 * np.cos(a2)
    ic[:, 0] = 1
    isn = -2 * np.sin(a2)
    isn[:, 0] = np.cos(np.pi * t[:, 0])
    inv = np.concatenate([ic, isn], 1) / (2 * C)
    inv2 = np.concatenate([inv[:C], inv[C:]], 1)
    return fw.astype(np.float32), inv2.astype(np.float32)


def _head(wref, hp, tr):
    w = wref[hp % 2]
    if tr:
        w = w.T
    lo = lax.bitcast_convert_type(w << 16, f32).astype(bf16)
    hi = lax.bitcast_convert_type(w & jnp.uint32(0xFFFF0000), f32).astype(bf16)
    return lo, hi


def _dot(a, b):
    return jnp.dot(a, b, preferred_element_type=f32)


def _kernel(aq_h, ak_h, av_h, sh, sk_h, sd, fw, inv, x, c, wq, wuk, wuv, wo, out,
            kvs, U, K, Z, cT, q_s, k_s, v_s, ctx_s, acc, wq_s, wk_s, wv_s, rq, rk, rv, sem, aq, ak, av, sk, sem2):
    p = pl.program_id(0)

    def fetch(i):
        return [pltpu.make_async_copy(w.bitcast(jnp.uint32).at[:, i, :], r.at[i % 2], sem.at[n])
                for n, (w, r) in enumerate(((wq, rq), (wuk, rk), (wuv, rv)))]

    a_in = [pltpu.make_async_copy(h_, v_, sem2.at[n])
            for n, (h_, v_) in enumerate(((aq_h, aq), (ak_h, ak), (av_h, av), (sk_h, sk)))]

    @pl.when(p == 0)
    def _():
        for cp in fetch(0):
            cp.start()
        for cp in a_in:
            cp.start()

        @pl.loop(0, NC)
        def _(ch):
            cs = pl.ds(pl.multiple_of(ch * C, C), C)
            cT[:, cs] = c[cs, :].T
            acc[:, cs] = jnp.zeros((M, C), f32)

    for cp in fetch(p):
        cp.wait()

    @pl.when(p + 1 < H // 2)
    def _():
        for cp in fetch(p + 1):
            cp.start()

    for src, dst, tr in ((rq, wq_s, True), (rk, wk_s, False), (rv, wv_s, True)):
        dst[0], dst[1] = _head(src, p, tr)
    wqs, wks, wvs = wq_s, wk_s, wv_s
    tri = (lax.broadcasted_iota(jnp.int32, (BQ, BQ), 0) <= lax.broadcasted_iota(jnp.int32, (BQ, BQ), 1))
    @pl.loop(0, 2)
    def _(e):
        for t in range(0, S, 512):
            r = slice(t, t + 512)
            q_s[:, r] = (_dot(wqs[e], x[:, r]) * (D ** -0.5)).astype(bf16)
            k_s[r, :] = _dot(c[r, :], wks[e]).astype(bf16)
            v_s[:, r] = _dot(wvs[e], cT[:, r]).astype(bf16)
        def qk(i):
            a, n = i * BQ, (i + 1) * BQ
            qi = q_s[:, a:n]
            hq = BQ // 2
            low = jnp.concatenate([jnp.zeros((hq, hq), f32), _dot(k_s[a + hq:n, :], qi[:, hq:])], 1)
            s1 = jnp.where(tri, jnp.concatenate([_dot(k_s[a:a + hq, :], qi), low], 0), -1e9)
            m = jnp.max(s1, 0, keepdims=True)
            s0 = None
            if i:
                s0 = _dot(k_s[:a, :], qi)
                m = jnp.maximum(m, jnp.max(s0, 0, keepdims=True))
            return s0, s1, m
        nxt = qk(0)
        for i in range(S // BQ):
            a, n = i * BQ, (i + 1) * BQ
            s0, s1, m = nxt
            if n < S:
                nxt = qk(i + 1)
            p1 = jnp.exp(s1 - m)
            l = jnp.sum(p1, 0, keepdims=True)
            pb, hq = p1.astype(bf16), BQ // 2
            o = jnp.concatenate([_dot(v_s[:, a:a + hq], pb[:hq, :hq]), _dot(v_s[:, a:n], pb[:, hq:])], 1)
            if i:
                p0 = jnp.exp(s0 - m)
                l = l + jnp.sum(p0, 0, keepdims=True)
                o = o + _dot(v_s[:, :a], p0.astype(bf16))
            ctx_s[:, a:n] = (o * (1.0 / l)).astype(bf16)
        for t in range(0, S, 512):
            r = slice(t, t + 512)
            acc[:, r] += _dot(wo[e], ctx_s[:, r])

    @pl.when(p == H // 2 - 1)
    def _():
        for cp in a_in:
            cp.wait()
        Z[0] = jnp.zeros((DA, 2 * C), bf16)
        F = fw[...]
        lane = lax.broadcasted_iota(jnp.int32, (DA, C), 1)

        @pl.loop(0, NC)
        def _(ch):
            cs = pl.ds(pl.multiple_of(ch * C, C), C)
            prev = ak[:, pl.ds(pl.multiple_of(jnp.maximum(ch - 1, 0) * C, C), C)].astype(f32)
            prev = jnp.where(ch > 0, prev, 0.0)
            cur = ak[:, cs].astype(f32)
            ks = jnp.zeros((DA, C), bf16)
            for j in (3, 2, 1, 0):
                kj = cur if j == 0 else pltpu.roll(jnp.where(lane >= C - j, prev, cur), j, 1)
                ks = ks + kj.astype(bf16) * sh[:, j:j + 1]
            kv = ks * av[:, cs]
            kvs[ch] = kv
            U[ch] = _dot(kv, F)
            kf = _dot(sk[:, cs], F)
            K[ch, :, :C] = kf[:, :C]
            K[ch, :, C:2 * C] = jnp.where(lane == 0, 0.0, kf[:, C:])
            K[ch, :, 2 * C:] = jnp.where(lane == 0, kf[:, C:], kf[:, :C])

        @pl.loop(0, DA // 16)
        def _(g):
            res = []
            for hf in range(2):
                rr = pl.ds(pl.multiple_of(g * 16 + hf * 8, 8), 8)
                zs = []
                for c0 in range(0, NC, 4):
                    z = [None] * 4
                    for j0 in range(0, c0 + 1, 4):
                        u = [(U[j, rr, :C], U[j, rr, C:]) for j in range(j0, j0 + 4)]
                        for d in range(max(c0 - j0 - 3, 0), c0 - j0 + 4):
                            k0, k1, k2 = K[d, rr, :C], K[d, rr, C:2 * C], K[d, rr, 2 * C:]
                            for i in range(4):
                                j = c0 + i - d - j0
                                if 0 <= j < 4:
                                    ur, ui = u[j]
                                    t = (k0 * ur - k1 * ui, k2 * ui + k1 * ur)
                                    z[i] = t if z[i] is None else (z[i][0] + t[0], z[i][1] + t[1])
                    zs += z
                res.append(zs)
            r16 = pl.ds(pl.multiple_of(g * 16, 16), 16)
            for ch in range(NC):
                for h in range(2):
                    Z[ch + 1, r16, h * C:(h + 1) * C] = jnp.concatenate(
                        [res[0][ch][h], res[1][ch][h]], 0).astype(bf16)

        @pl.loop(0, S // 256)
        def _(t):
            r = pl.ds(pl.multiple_of(t * 256, 256), 256)
            out[r, DA:] = acc[:, r].T.astype(bf16)
            for u in range(2):
                ch = 2 * t + u
                y = (_dot(Z[ch + 1], inv[:2 * C, :]) + _dot(Z[ch], inv[2 * C:, :])).astype(bf16)
                rc = pl.ds(pl.multiple_of(ch * C, C), C)
                y = y + kvs[ch] * sd[...]
                out[rc, :DA] = (aq[:, rc] * y).astype(f32).T.astype(bf16)


@jax.jit
def pallas_concat_heads__ssm_conv_h3__compressed_kv_cla__prompt_kernel(
        A_q, A_k, A_v, A_shift_k, A_ssm_k, A_ssm_D, B_x, B_c_kv, B_w_q, B_w_uk, B_w_uv, B_w_o):
    fw, inv = _dft()
    fw, inv = jnp.asarray(fw.T, bf16), jnp.asarray(inv.T, bf16)

    def full(a):
        nd = a.ndim
        return pl.BlockSpec(a.shape, lambda p: (0,) * nd, pipeline_mode=pl.Buffered(1))
    args = [A_q[0].T, A_k[0].T, A_v[0].T, A_shift_k, A_ssm_k, A_ssm_D[:, None], fw, inv,
            B_x[0].T, B_c_kv[0]]
    V = pltpu.VMEM
    o = pl.pallas_call(
        _kernel,
        grid=(H // 2,),
        in_specs=[pl.BlockSpec(memory_space=pl.ANY) if n in (0, 1, 2, 4) else full(a)
                  for n, a in enumerate(args)] + [pl.BlockSpec(memory_space=pl.ANY)] * 3 + [pl.BlockSpec((2, M, D), lambda p: (p, 0, 0))],
        out_specs=pl.BlockSpec((S, DA + M), lambda p: (0, 0)),
        out_shape=jax.ShapeDtypeStruct((S, DA + M), bf16),
        scratch_shapes=[V((NC, DA, C), bf16), V((NC, DA, 2 * C), f32),
                        V((NC, DA, 3 * C), f32), V((NC + 1, DA, 2 * C), bf16), V((DC, S), bf16),
                        V((D, S), bf16), V((S, D), bf16), V((D, S), bf16),
                        V((D, S), bf16), V((M, S), f32),
                        V((2, D, M), bf16), V((2, DC, D), bf16), V((2, D, DC), bf16),
                        V((2, M, D), jnp.uint32), V((2, DC, D), jnp.uint32), V((2, DC, D), jnp.uint32),
                        pltpu.SemaphoreType.DMA((3,))] + [V((DA, S), bf16)] * 4 + [pltpu.SemaphoreType.DMA((4,))],
        compiler_params=pltpu.CompilerParams(dimension_semantics=("arbitrary",),
                                             flags={"XLA_TPU_FORCE_LP_LLO_SCHEDULER": False}, vmem_limit_bytes=120 * 2 ** 20),
    )(*args, B_w_q, B_w_uk, B_w_uv, B_w_o.transpose(0, 2, 1))
    return o[None]
```
